```python
import os as _os
_os.environ.setdefault("JAX_PLATFORMS", "cpu")
import jax
import jax.numpy as jnp

def _softmax(x, axis=-1):
    return jax.nn.softmax(x, axis=axis)
def _gelu(x):
    return jax.nn.gelu(x, approximate=True)
def _silu(x):
    return jax.nn.silu(x)
def _sigmoid(x):
    return jax.nn.sigmoid(x)
def _layernorm(x, axis=-1, eps=1e-5):
    m = jnp.mean(x, axis=axis, keepdims=True)
    v = jnp.var(x, axis=axis, keepdims=True)
    return (x - m) / jnp.sqrt(v + eps)
def _scatter_add(tgt, idx, src, axis=0):
    return tgt.at[idx].add(src)
def _segment_sum(src, seg, n):
    return jax.ops.segment_sum(src, seg, n)
class _Rng:
    def __init__(self, key):
        self._k = key
    def _next(self):
        self._k, sub = jax.random.split(self._k)
        return sub
    def normal(self, shape):
        return jax.random.normal(self._next(), shape, dtype=jnp.bfloat16)
    def randint(self, lo, hi, shape):
        return jax.random.randint(self._next(), shape, lo, hi, dtype=jnp.int32)
    def uniform(self, shape, lo=0.0, hi=1.0):
        return jax.random.uniform(self._next(), shape, jnp.bfloat16, lo, hi)
    def permutation(self, n):
        return jax.random.permutation(self._next(), n)


kernel_name = 'sequential_preLN__mha_block__dense_activation_mish__prompt'

def setup_inputs():
    _rng = _Rng(jax.random.key(int.from_bytes(__import__("os").urandom(4), "little")))
    _w = (lambda a: (lambda t: t.astype(jnp.bfloat16) if jnp.issubdtype(t.dtype, jnp.floating) else t)(jnp.asarray(a)))
    def _A_setup():
        B, S, D, H = 1, 2048, 576, 32
        return {
            "x": _w((lambda *s: _rng.normal(s) * 0.05)(B, S, D)),
            "wqkv": _w((lambda *s: _rng.normal(s) * 0.05)(D, 3 * D)),
            "wo": _w((lambda *s: _rng.normal(s) * 0.05)(D, D)),
        }
    _A_in = _A_setup()

    def _B_setup():
        B, S, D, F = 1, 2048, 576, 4608
        return {
            "x": _w((lambda *s: _rng.normal(s) * 0.05)(B, S, D)),
            "w1": _w((lambda *s: _rng.normal(s) * 1.6)(D, F) * (D ** -0.5)),
            "b1": _w((lambda *s: _rng.normal(s) * 0.05)(F)),
            "w2": _w((lambda *s: _rng.normal(s) * 0.05)(F, D) * (F ** -0.5)),
        }
    _B_in = _B_setup()

    return {
        "A_x": _A_in["x"],
        "A_wqkv": _A_in["wqkv"],
        "A_wo": _A_in["wo"],
        "B_x": _B_in["x"],
        "B_w1": _B_in["w1"],
        "B_b1": _B_in["b1"],
        "B_w2": _B_in["w2"],
    }

def reference(A_x, A_wqkv, A_wo, B_x, B_w1, B_b1, B_w2):
    def _A_ref(x, wqkv, wo):
        B, S, D = x.shape
        H = 32
        Dh = D // H
        qkv = (lambda x, *d: x.transpose(*d))((x @ wqkv).reshape(B, S, 3, H, Dh), 2, 0, 3, 1, 4)
        q, k, v = qkv[0], qkv[1], qkv[2]
        scores = jnp.einsum("bhqd,bhkd->bhqk", q, k) * (Dh ** -0.5)
        p = _softmax(scores, axis=-1)
        o = jnp.einsum("bhqk,bhkd->bhqd", p, v)
        return (lambda x, *d: x.transpose(*d))(o, 0, 2, 1, 3).reshape(B, S, D) @ wo

    def _B_ref(x, w1, b1, w2):
        h = jnp.einsum("bsd,df->bsf", x, w1) + b1
        sp = jnp.log1p(jnp.exp(-jnp.abs(h))) + jnp.where(h > 0, h, jnp.zeros_like(h))
        act = h * jnp.tanh(sp)
        return jnp.einsum("bsf,fd->bsd", act, w2)

    x = A_x
    h = x + _A_ref(_layernorm(x, axis=-1), A_wqkv, A_wo)
    h2 = h + _B_ref(_layernorm(h, axis=-1), B_w1, B_b1, B_w2)
    return h2
```

```python
import jax
import jax.numpy as jnp
from jax import lax
import jax.experimental.pallas as pl
import jax.experimental.pallas.tpu as pltpu

S = 2048
D = 576
H = 32
DH = 18
F = 4608
HPG = 7
NG = 5
VP = 32
TQ = 512
NQ = S // TQ
FC = 2304
EPS = 1e-5
_NT = (((1,), (1,)), ((), ()))
_TN = (((0,), (0,)), ((), ()))


def _layernorm_t(x):
    m = jnp.mean(x, axis=0, keepdims=True)
    xc = x - m
    v = jnp.mean(xc * xc, axis=0, keepdims=True)
    return xc * lax.rsqrt(v + EPS)


def _mish(h):
    sp = jnp.log1p(jnp.exp(-jnp.abs(h))) + jnp.maximum(h, 0.0)
    return h * jnp.tanh(sp)


def _kernel(xt_hbm, wqkv_ref, wo_hbm, w1_hbm, b1_ref, w2t_hbm, o_ref,
            k_scr, qt_scr, vt_scr, ot_scr, oc_scr, s_scr, m_scr, wot_scr,
            wkp_scr, wqt_scr, wvt_scr, w1_ref, w2t_ref, xt_ref, wo_ref,
            sems):
    i = pl.program_id(0)
    bf16 = jnp.bfloat16
    f32 = jnp.float32

    @pl.when(i == 0)
    def _phase1():
        pltpu.make_async_copy(xt_hbm, xt_ref, sems.at[2]).start()
        pltpu.make_async_copy(wo_hbm, wo_ref, sems.at[3]).start()
        pltpu.make_async_copy(w1_hbm, w1_ref, sems.at[0]).start()
        pltpu.make_async_copy(w2t_hbm, w2t_ref, sems.at[1]).start()
        scale = DH ** -0.5
        GW = HPG * DH
        wkp_scr[...] = jnp.zeros_like(wkp_scr)
        wqt_scr[...] = jnp.zeros_like(wqt_scr)
        wk = wqkv_ref[:, D:2 * D].astype(f32)
        wq_t = wqkv_ref[:, 0:D].astype(f32).T
        for g in range(NG):
            n = min(GW, D - g * GW)
            wkp_scr[:, g * 128:g * 128 + n] = (
                wk[:, g * GW:g * GW + n].astype(bf16))
            wqt_scr[g * 128:g * 128 + n, :] = (
                wq_t[g * GW:g * GW + n, :].astype(bf16))
        wvt_scr[...] = wqkv_ref[:, 2 * D:3 * D].astype(f32).T.astype(bf16)
        pltpu.make_async_copy(wo_hbm, wo_ref, sems.at[3]).wait()
        wot_scr[...] = wo_ref[...].astype(f32).T.astype(bf16)
        pltpu.make_async_copy(xt_hbm, xt_ref, sems.at[2]).wait()
        row = lax.broadcasted_iota(jnp.int32, (H * VP, S), 0)
        vt_scr[...] = jnp.where((row % VP) == DH, 1.0, 0.0).astype(bf16)

        def blk(j, carry):
            off = pl.multiple_of(j * TQ, TQ)
            xnt = _layernorm_t(xt_ref[:, pl.ds(off, TQ)].astype(f32)
                               ).astype(bf16)
            kj = lax.dot_general(xnt, wkp_scr[...], _TN,
                                 preferred_element_type=f32)
            for g in range(NG):
                k_scr[g, pl.ds(off, TQ), :] = (
                    kj[:, g * 128:(g + 1) * 128].astype(bf16))
            qt = jnp.dot(wqt_scr[...], xnt, preferred_element_type=f32)
            for g in range(NG):
                qt_scr[j, g] = (qt[g * 128:(g + 1) * 128, :] * scale
                                ).astype(bf16)
            vt = jnp.dot(wvt_scr[...], xnt, preferred_element_type=f32)
            for hh in range(H):
                vt_scr[hh * VP:hh * VP + DH, pl.ds(off, TQ)] = (
                    vt[hh * DH:(hh + 1) * DH, :].astype(bf16))
            return carry

        lax.fori_loop(0, NQ, blk, 0)

    rowq = lax.broadcasted_iota(jnp.int32, (128, TQ), 0)

    def scores(h, blk, slot):
        g = h // HPG
        lo = (h - g * HPG) * DH
        qt = qt_scr[blk, g]
        qm = jnp.where((rowq >= lo) & (rowq < lo + DH), qt, jnp.zeros_like(qt))
        s = jnp.dot(k_scr[g], qm, preferred_element_type=f32)
        s_scr[slot] = s
        m_scr[slot] = jnp.max(s, axis=0, keepdims=True)

    def finish(h, slot):
        p = jnp.exp(s_scr[slot] - m_scr[slot]).astype(bf16)
        off = pl.multiple_of(h * VP, VP)
        vt = vt_scr[pl.ds(off, VP), :]
        o = jnp.dot(vt, p, preferred_element_type=f32)
        inv = 1.0 / o[DH:DH + 1, :]
        ot_scr[pl.ds(off, VP), :] = o * inv

    @pl.when(i == 0)
    def _first_scores():
        scores(0, 0, 0)

    def pair_body(t, carry):
        h = 2 * t
        scores(h + 1, i, 1)
        finish(h, 0)
        wrap = h + 2 >= H
        scores(jnp.where(wrap, 0, h + 2),
               jnp.where(wrap, jnp.minimum(i + 1, NQ - 1), i), 0)
        finish(h + 1, 1)
        return carry

    lax.fori_loop(0, H // 2, pair_body, 0)

    for hh in range(H):
        oc_scr[hh * DH:(hh + 1) * DH, :] = ot_scr[hh * VP:hh * VP + DH, :]
    attn_t = jnp.dot(wot_scr[...], oc_scr[...].astype(bf16),
                     preferred_element_type=f32)
    start = pl.multiple_of(i * TQ, TQ)
    hres_t = xt_ref[:, pl.ds(start, TQ)].astype(f32) + attn_t
    hn = _layernorm_t(hres_t).T.astype(bf16)

    @pl.when(i == 0)
    def _wait_weights():
        pltpu.make_async_copy(w1_hbm, w1_ref, sems.at[0]).wait()
        pltpu.make_async_copy(w2t_hbm, w2t_ref, sems.at[1]).wait()

    def mlp_body(c, acc):
        off = pl.multiple_of(c * FC, FC)
        a = jnp.dot(hn, w1_ref[:, pl.ds(off, FC)], preferred_element_type=f32)
        a = a + b1_ref[:, pl.ds(off, FC)].astype(f32)
        act = _mish(a).astype(bf16)
        return acc + lax.dot_general(act, w2t_ref[:, pl.ds(off, FC)], _NT,
                                     preferred_element_type=f32)

    acc = lax.fori_loop(0, F // FC, mlp_body, jnp.zeros((TQ, D), f32))
    o_ref[...] = (hres_t + acc.T).astype(o_ref.dtype)


@jax.jit
def pallas_sequential_preLN__mha_block__dense_activation_mish__prompt_kernel(
    A_x, A_wqkv, A_wo, B_x, B_w1, B_b1, B_w2,
):
    del B_x
    xt = A_x.reshape(S, D).T
    b1 = B_b1.reshape(1, F)
    w2t = B_w2.T

    const = lambda i: (0, 0)
    out_t = pl.pallas_call(
        _kernel,
        grid=(NQ,),
        in_specs=[
            pl.BlockSpec(memory_space=pl.ANY),
            pl.BlockSpec((D, 3 * D), const),
            pl.BlockSpec(memory_space=pl.ANY),
            pl.BlockSpec(memory_space=pl.ANY),
            pl.BlockSpec((1, F), const),
            pl.BlockSpec(memory_space=pl.ANY),
        ],
        out_specs=pl.BlockSpec((D, TQ), lambda i: (0, i)),
        out_shape=jax.ShapeDtypeStruct((D, S), jnp.bfloat16),
        scratch_shapes=[
            pltpu.VMEM((NG, S, 128), jnp.bfloat16),
            pltpu.VMEM((NQ, NG, 128, TQ), jnp.bfloat16),
            pltpu.VMEM((H * VP, S), jnp.bfloat16),
            pltpu.VMEM((H * VP, TQ), jnp.float32),
            pltpu.VMEM((D, TQ), jnp.float32),
            pltpu.VMEM((2, S, TQ), jnp.float32),
            pltpu.VMEM((2, 1, TQ), jnp.float32),
            pltpu.VMEM((D, D), jnp.bfloat16),
            pltpu.VMEM((D, NG * 128), jnp.bfloat16),
            pltpu.VMEM((NG * 128, D), jnp.bfloat16),
            pltpu.VMEM((D, D), jnp.bfloat16),
            pltpu.VMEM((D, F), jnp.bfloat16),
            pltpu.VMEM((D, F), jnp.bfloat16),
            pltpu.VMEM((D, S), jnp.bfloat16),
            pltpu.VMEM((D, D), jnp.bfloat16),
            pltpu.SemaphoreType.DMA((4,)),
        ],
        compiler_params=pltpu.CompilerParams(
            dimension_semantics=("arbitrary",),
            vmem_limit_bytes=100 * 1024 * 1024,
        ),
    )(xt, A_wqkv, A_wo, B_w1, b1, w2t)
    return out_t.T.reshape(1, S, D)
```
